```python
import jax
import jax.numpy as jnp

def _softmax(x, axis=-1):
    return jax.nn.softmax(x, axis=axis)
def _gelu(x):
    return jax.nn.gelu(x, approximate=True)
def _silu(x):
    return jax.nn.silu(x)
def _sigmoid(x):
    return jax.nn.sigmoid(x)
def _layernorm(x, axis=-1, eps=1e-5):
    m = jnp.mean(x, axis=axis, keepdims=True)
    v = jnp.var(x, axis=axis, keepdims=True)
    return (x - m) / jnp.sqrt(v + eps)
def _scatter_add(tgt, idx, src, axis=0):
    return tgt.at[idx].add(src)
def _segment_sum(src, seg, n):
    return jax.ops.segment_sum(src, seg, n)
class _Rng:
    def __init__(self, key):
        self._k = key
    def _next(self):
        self._k, sub = jax.random.split(self._k)
        return sub
    def normal(self, shape):
        return jax.random.normal(self._next(), shape, dtype=jnp.bfloat16)
    def randint(self, lo, hi, shape):
        return jax.random.randint(self._next(), shape, lo, hi, dtype=jnp.int32)
    def uniform(self, shape, lo=0.0, hi=1.0):
        return jax.random.uniform(self._next(), shape, jnp.bfloat16, lo, hi)
    def permutation(self, n):
        return jax.random.permutation(self._next(), n)


kernel_name = 'gated_mix__compressed_kv_cla__sliding_local_dilated__prompt'

def setup_inputs():
    _rng = _Rng(jax.random.key(int.from_bytes(__import__("os").urandom(4), "little")))
    _w = (lambda a: (lambda t: t.astype(jnp.bfloat16) if jnp.issubdtype(t.dtype, jnp.floating) else t)(jnp.asarray(a)))
    def _A_setup():
        B, H, Sq, Sk, D, M = 1, 32, 2048, 2048, 128, 1024
        Dc = 4 * D
        return {
            "x": _w((lambda *s: _rng.normal(s) * 0.05)(B, Sq, M)),
            "c_kv": _w((lambda *s: _rng.normal(s) * 0.05)(B, Sk, Dc)),
            "w_q": _w((lambda *s: _rng.normal(s) * 0.05)(M, H, D) * (M ** -0.5)),
            "w_uk": _w((lambda *s: _rng.normal(s) * 0.05)(Dc, H, D) * (Dc ** -0.5)),
            "w_uv": _w((lambda *s: _rng.normal(s) * 0.05)(Dc, H, D) * (Dc ** -0.5)),
            "w_o": _w((lambda *s: _rng.normal(s) * 0.05)(H, D, M) * ((H * D) ** -0.5)),
        }
    _A_in = _A_setup()

    def _B_setup():
        B, S, D = 1, 2048, 1024
        return {
            "x": _w((lambda *s: _rng.normal(s) * 0.05)(B, S, D)),
            "wqkv": _w((lambda *s: _rng.normal(s) * 0.05)(D, 3 * D)),
            "wo": _w((lambda *s: _rng.normal(s) * 0.05)(D, D)),
        }
    _B_in = _B_setup()

    return {
        "A_x": _A_in["x"],
        "A_c_kv": _A_in["c_kv"],
        "A_w_q": _A_in["w_q"],
        "A_w_uk": _A_in["w_uk"],
        "A_w_uv": _A_in["w_uv"],
        "A_w_o": _A_in["w_o"],
        "B_x": _B_in["x"],
        "B_wqkv": _B_in["wqkv"],
        "B_wo": _B_in["wo"],
        "gate_w": _w((lambda *s: _rng.normal(s) * 0.05)(1024)),
    }

def reference(A_x, A_c_kv, A_w_q, A_w_uk, A_w_uv, A_w_o, B_x, B_wqkv, B_wo, gate_w):
    def _A_ref(x, c_kv, w_q, w_uk, w_uv, w_o):
        B, Sq, M = x.shape[0], x.shape[1], x.shape[2]
        Sk = c_kv.shape[1]
        H, D = w_q.shape[1], w_q.shape[2]
        q = jnp.einsum("bqm,mhd->bhqd", x, w_q)
        k = jnp.einsum("bkc,chd->bhkd", c_kv, w_uk)
        v = jnp.einsum("bkc,chd->bhkd", c_kv, w_uv)
        scores = jnp.einsum("bhqd,bhkd->bhqk", q, k) * (D ** -0.5)
        off = Sk - Sq
        qi = jnp.arange(Sq)[:, None]
        kj = jnp.arange(Sk)[None, :]
        cmask = kj <= (qi + off)
        scores = jnp.where(cmask[None, None], scores, -1e9)
        p = _softmax(scores, axis=-1)
        ctx = jnp.einsum("bhqk,bhkd->bhqd", p, v)
        return jnp.einsum("bhqd,hdm->bqm", ctx, w_o)

    def _B_ref(x, wqkv, wo):
        B, S, D = x.shape
        H = 32; Dh = D // H
        W, dil = 8, 2
        qkv = (lambda x, *d: x.transpose(*d))((x @ wqkv).reshape(B, S, 3, H, Dh), 2, 0, 3, 1, 4)
        q, k, v = qkv[0], qkv[1], qkv[2]
        scale = Dh ** -0.5
        pos = jnp.arange(S)
        off = jnp.arange(W) * dil
        idx = pos[:, None] - off[None, :]
        mask = idx >= 0
        idx_c = jnp.where(mask, idx, 0).reshape(-1)
        kg = k[:, :, idx_c, :].reshape(B, H, S, W, Dh)
        vg = v[:, :, idx_c, :].reshape(B, H, S, W, Dh)
        logits = jnp.einsum("bhsd,bhswd->bhsw", q, kg) * scale
        logits = jnp.where(mask[None, None, :, :], logits, -1e9)
        attn = _softmax(logits, axis=-1)
        o = jnp.einsum("bhsw,bhswd->bhsd", attn, vg)
        return (lambda x, *d: x.transpose(*d))(o, 0, 2, 1, 3).reshape(B, S, D) @ wo

    x = A_x
    g = _sigmoid((x * gate_w).sum(-1, keepdims=True))
    a = _A_ref(x, A_c_kv, A_w_q, A_w_uk, A_w_uv, A_w_o)
    b = _B_ref(x, B_wqkv, B_wo)
    return g * a + (1 - g) * b
```

```python
import functools
import math

import jax
import jax.numpy as jnp
import numpy as np
import jax.experimental.pallas as pl
import jax.experimental.pallas.tpu as pltpu

_LOG2E = math.log2(math.e)
_NT = (((1,), (1,)), ((), ()))
_NEG = -1e9 * _LOG2E


def _merge(*lists):
    items = []
    for li, lst in enumerate(lists):
        n = len(lst)
        for k, t in enumerate(lst):
            items.append(((k + 0.5) / n, li, k, t))
    items.sort(key=lambda e: (e[0], e[1], e[2]))
    return [e[3] for e in items]


def _kernel(x_hbm, c_hbm, wq_hbm, wuk_hbm, wuv_hbm, wo_hbm, wqkv_hbm, wob_hbm, gw_ref,
            o_hbm,
            x_s, c_s, wq_raw, wuk_raw, wuv_raw, wo_s, wqkv_s, wob_s,
            wq_s, wuk_s, wuv_s, acc_s, g_s, q_s, k_s, v_s, s_s, m_s, p_s, r_s, ctx_s, kh_s, vh_s, ostage, sems,
            *, S, H, D, HB, DB, W, DIL, BQ, RB, CK, NC, RS, FILL_AT, CKV):
    step = pl.program_id(0)
    f32, bf16, u32 = jnp.float32, jnp.bfloat16, jnp.uint32
    NB = S // RB
    M = x_s.shape[1]
    DM = HB * DB
    HALO = 16

    def cp(i):
        srcs = [
            (x_hbm.at[pl.ds(0, RB)], x_s.at[pl.ds(0, RB)]),
            (wqkv_hbm, wqkv_s),
            (x_hbm.at[pl.ds(RB, S - RB)], x_s.at[pl.ds(RB, S - RB)]),
            (wob_hbm, wob_s),
            (c_hbm, c_s),
            (wuk_hbm, wuk_raw),
            (wuv_hbm, wuv_raw),
            (wq_hbm, wq_raw),
            (wo_hbm, wo_s),
        ]
        s, d = srcs[i]
        return pltpu.make_async_copy(s, d, sems.at[i])

    GH = 8
    NCH = GH

    def prep_weights(grp, src_grp, ch):
        slot = grp & 1
        thunks = []
        for raw, dst in ((wq_raw, wq_s), (wuk_raw, wuk_s), (wuv_raw, wuv_s)):
            rows = dst.shape[2] // NCH
            base = pl.multiple_of(ch * (rows * (H // 2)) + src_grp * (GH // 2), GH // 2)
            d0 = pl.multiple_of(ch * rows, rows)
            for b in range(GH // 2):
                def t(raw=raw, dst=dst, rows=rows, base=base, d0=d0, b=b):
                    w32 = raw.bitcast(u32).at[pl.ds(base, rows * (H // 2) - (H - GH) // 2)][pl.ds(b, rows, stride=H // 2), :]
                    lo = pltpu.bitcast(w32 << 16, f32).astype(bf16)
                    hi = pltpu.bitcast(w32 & u32(0xFFFF0000), f32).astype(bf16)
                    dst[slot, 2 * b, pl.ds(d0, rows), :] = lo
                    dst[slot, 2 * b + 1, pl.ds(d0, rows), :] = hi
                thunks.append(t)
        return thunks

    @pl.when(step == 0)
    def _():
        cp(0).start()
        cp(1).start()
        cp(0).wait()
        cp(1).wait()
        for i in range(2, 9):
            cp(i).start()
        kh_s[RB:RB + HALO, :] = jnp.zeros((HALO, M), f32)
        vh_s[RB:RB + HALO, :] = jnp.zeros((HALO, M), f32)

    @pl.when(step == 1)
    def _():
        cp(2).wait()

    @pl.when(step < NB)
    def _():
        r0 = pl.multiple_of(step * RB, RB)
        xb = x_s[pl.ds(r0, RB), :]
        z = jnp.sum(xb.astype(f32) * gw_ref[...].astype(f32), axis=-1, keepdims=True)
        g = jnp.broadcast_to(jax.nn.sigmoid(z), (RB, 128))
        g_s[pl.ds(r0, RB), :] = g
        q = jnp.dot(xb, wqkv_s[:, 0:DM], preferred_element_type=f32) * ((DB ** -0.5) * _LOG2E)
        kh_s[0:HALO, :] = kh_s[RB:RB + HALO, :]
        vh_s[0:HALO, :] = vh_s[RB:RB + HALO, :]
        kh_s[HALO:HALO + RB, :] = jnp.dot(xb, wqkv_s[:, DM:2 * DM], preferred_element_type=f32)
        vh_s[HALO:HALO + RB, :] = jnp.dot(xb, wqkv_s[:, 2 * DM:3 * DM], preferred_element_type=f32)
        li = jax.lax.broadcasted_iota(jnp.int32, (128, 128), 0) // DB
        lj = jax.lax.broadcasted_iota(jnp.int32, (128, 128), 1) // DB
        ones_bd = (li == lj).astype(bf16)
        pos = r0 + jax.lax.broadcasted_iota(jnp.int32, (RB, 128), 0)
        outs = []
        for cidx in range(DM // 128):
            cs = slice(cidx * 128, (cidx + 1) * 128)
            qc = q[:, cs]
            logits = []
            for w in range(W):
                kw = kh_s[HALO - w * DIL:HALO - w * DIL + RB, cs]
                lg = jnp.dot((qc * kw).astype(bf16), ones_bd, preferred_element_type=f32)
                if w > 0:
                    lg = jnp.where(pos >= w * DIL, lg, _NEG)
                logits.append(lg)
            m = logits[0]
            for w in range(1, W):
                m = jnp.maximum(m, logits[w])
            ps = [jnp.exp2(lg - m) for lg in logits]
            l = ps[0]
            for w in range(1, W):
                l = l + ps[w]
            o = ps[0] * vh_s[HALO:HALO + RB, cs]
            for w in range(1, W):
                o = o + ps[w] * vh_s[HALO - w * DIL:HALO - w * DIL + RB, cs]
            outs.append((o * ((1.0 - g) / l)).astype(bf16))
        ob = jnp.concatenate(outs, axis=-1)

        @pl.when(step == 0)
        def _():
            cp(3).wait()

        acc_s[pl.ds(r0, RB), :] = jnp.dot(ob, wob_s[...], preferred_element_type=f32)

    @pl.when(step == NB - 1)
    def _():
        for i in range(4, 9):
            cp(i).wait()
        def body(ch, carry):
            for t in prep_weights(0, 0, ch):
                t()
            return carry
        jax.lax.fori_loop(0, NCH, body, 0)

    @pl.when(step >= NB)
    def _():
        h = step - NB
        slot = (h >> 3) & 1
        hh = h & 7
        qscale = (D ** -0.5) * _LOG2E
        q_s[...] = (jnp.dot(x_s[...], wq_s[slot, hh], preferred_element_type=f32) * qscale).astype(bf16)
        c = c_s[...]
        k_s[...] = jnp.dot(c, wuk_s[slot, hh], preferred_element_type=f32).astype(bf16)
        v_s[...] = jnp.dot(c, wuv_s[slot, hh], preferred_element_type=f32).astype(bf16)
        wo_h = wo_s.at[pl.ds(pl.multiple_of(h * D, D), D), :]
        fill = prep_weights((h >> 3) + 1, jnp.minimum((h >> 3) + 1, H // GH - 1), hh)

        HF = BQ // 2
        row = jax.lax.broadcasted_iota(jnp.int32, (HF, HF), 0)
        col = jax.lax.broadcasted_iota(jnp.int32, (HF, HF), 1)
        cmask = col <= row
        nq = S // BQ
        st = [dict() for _ in range(nq)]

        def upd(d, key, val):
            d[key] = val if not (key in d) else d[key] + val

        def tmax(a):
            r = a[:, 0:128]
            for t in range(1, a.shape[1] // 128):
                r = jnp.maximum(r, a[:, t * 128:(t + 1) * 128])
            return r

        def ptiles(slot, a0, a1, c0, c1):
            return jnp.concatenate([p_s[slot, c, a0:a1, :] for c in range(c0 // 128, c1 // 128)], axis=1)

        def stage_a(i):
            r0 = i * BQ
            th = []
            nmx = 0
            for c0 in range(0, r0, CK):
                def t(c0=c0, nmx=nmx):
                    ck = min(CK, r0 - c0)
                    s = jax.lax.dot_general(q_s[r0:r0 + BQ, :], k_s[c0:c0 + ck, :], _NT,
                                            preferred_element_type=f32)
                    s_s[i % 2, :, c0:c0 + ck] = s
                    m_s[i % 2, nmx] = tmax(s)
                th.append(t)
                nmx += 1

            def td1(nmx=nmx):
                s1 = jax.lax.dot_general(q_s[r0:r0 + HF, :], k_s[r0:r0 + HF, :], _NT,
                                         preferred_element_type=f32)
                s1 = jnp.where(cmask, s1, _NEG)
                s_s[i % 2, 0:HF, r0:r0 + HF] = s1
                m_s[i % 2, nmx, 0:HF, :] = s1

            def td2(nmx=nmx):
                s2 = jax.lax.dot_general(q_s[r0 + HF:r0 + BQ, :], k_s[r0:r0 + BQ, :], _NT,
                                         preferred_element_type=f32)
                s2b = jnp.where(cmask, s2[:, HF:BQ], _NEG)
                s_s[i % 2, HF:BQ, r0:r0 + HF] = s2[:, 0:HF]
                s_s[i % 2, HF:BQ, r0 + HF:r0 + BQ] = s2b
                m_s[i % 2, nmx, HF:BQ, :] = jnp.maximum(s2[:, 0:HF], s2b)
            return th + [td1, td2]

        def stage_sm(i):
            r0 = i * BQ
            th = []
            nmx = (r0 + CK - 1) // CK + 1
            for a0 in range(0, BQ, RS):
                def t(a0=a0):
                    L = r0 + (HF if a0 < HF else BQ)
                    nt = L // 128
                    m = m_s[i % 2, 0, a0:a0 + RS, :]
                    for c in range(1, nmx):
                        m = jnp.maximum(m, m_s[i % 2, c, a0:a0 + RS, :])
                    m = jnp.max(m, axis=-1, keepdims=True)
                    l = None
                    for c in range(nt):
                        p = jnp.exp2(s_s[i % 2, a0:a0 + RS, c * 128:(c + 1) * 128] - m)
                        l = p if l is None else l + p
                        p_s[i % 2, c, a0:a0 + RS, :] = p.astype(bf16)
                    l = jnp.sum(l, axis=-1, keepdims=True)
                    r_s[i % 2, a0:a0 + RS, :] = g_s[r0 + a0:r0 + a0 + RS, :] / l
                th.append(t)
            return th

        def stage_pv(i):
            r0 = i * BQ
            d = st[i]
            th = []
            for c0 in range(0, r0, CKV):
                def t(c0=c0):
                    ck = min(CKV, r0 - c0)
                    upd(d, 'o', jnp.dot(ptiles(i % 2, 0, BQ, c0, c0 + ck), v_s[c0:c0 + ck, :],
                                        preferred_element_type=f32))
                th.append(t)

            def td():
                o1 = jnp.dot(ptiles(i % 2, 0, HF, r0, r0 + HF), v_s[r0:r0 + HF, :], preferred_element_type=f32)
                o2 = jnp.dot(ptiles(i % 2, HF, BQ, r0, r0 + BQ), v_s[r0:r0 + BQ, :], preferred_element_type=f32)
                upd(d, 'o', jnp.concatenate([o1, o2], axis=0))
                ctx_s[i % 2] = (d['o'] * r_s[i % 2]).astype(bf16)
            return th + [td]

        def stage_c(i):
            r0 = i * BQ
            th = []
            for n0 in range(0, M, NC):
                def t(n0=n0):
                    acc_s[r0:r0 + BQ, n0:n0 + NC] += jnp.dot(ctx_s[i % 2], wo_h[:, n0:n0 + NC],
                                                             preferred_element_type=f32)
                th.append(t)
            return th

        prog = []
        for t_ in range(nq + 3):
            lists = []
            if t_ < nq:
                lists.append(stage_a(t_))
            if 0 <= t_ - 1 < nq:
                lists.append(stage_sm(t_ - 1))
            if 0 <= t_ - 2 < nq:
                lists.append(stage_pv(t_ - 2))
            if 0 <= t_ - 3 < nq:
                lists.append(stage_c(t_ - 3))
            if t_ == FILL_AT:
                lists.append(fill)
            prog += _merge(*lists)
        for t in prog:
            t()

    @pl.when(step == NB + H - 1)
    def _():
        def ocp(b):
            return pltpu.make_async_copy(ostage.at[b], o_hbm.at[pl.ds(b * RB, RB)], sems.at[9 + b])
        for b in range(NB):
            ostage[b] = acc_s[b * RB:(b + 1) * RB, :].astype(bf16)
            ocp(b).start()
        for b in range(NB):
            ocp(b).wait()


@jax.jit
def pallas_gated_mix__compressed_kv_cla__sliding_local_dilated__prompt_kernel(
    A_x: jax.Array,
    A_c_kv: jax.Array,
    A_w_q: jax.Array,
    A_w_uk: jax.Array,
    A_w_uv: jax.Array,
    A_w_o: jax.Array,
    B_x: jax.Array,
    B_wqkv: jax.Array,
    B_wo: jax.Array,
    gate_w: jax.Array,
):
    B, S, M = A_x.shape
    _, H, D = A_w_q.shape
    Dc = A_c_kv.shape[2]
    HB = 32
    DB = M // HB
    W, DIL = 8, 2
    BQ, RB = 256, 256
    CK, CKV, NC, RS, FILL_AT = 512, 1024, 512, 32, 5
    NB = S // RB
    f32, bf16 = jnp.float32, jnp.bfloat16

    x = A_x.reshape(S, M)
    c = A_c_kv.reshape(S, Dc)
    wq = A_w_q.reshape(M * H, D)
    wuk = A_w_uk.reshape(Dc * H, D)
    wuv = A_w_uv.reshape(Dc * H, D)
    wo = A_w_o.reshape(H * D, M)
    gw = gate_w.reshape(1, M)

    hbm = pl.BlockSpec(memory_space=pltpu.HBM)
    kern = functools.partial(_kernel, S=S, H=H, D=D, HB=HB, DB=DB, W=W, DIL=DIL, BQ=BQ, RB=RB,
                             CK=CK, NC=NC, RS=RS, FILL_AT=FILL_AT, CKV=CKV)
    out = pl.pallas_call(
        kern,
        grid=(NB + H,),
        in_specs=[hbm] * 8 + [pl.BlockSpec((1, M), lambda s: (0, 0))],
        out_specs=hbm,
        out_shape=jax.ShapeDtypeStruct((S, M), A_x.dtype),
        scratch_shapes=[
            pltpu.VMEM((S, M), bf16),
            pltpu.VMEM((S, Dc), bf16),
            pltpu.VMEM((M * H, D), bf16),
            pltpu.VMEM((Dc * H, D), bf16),
            pltpu.VMEM((Dc * H, D), bf16),
            pltpu.VMEM((H * D, M), bf16),
            pltpu.VMEM((M, 3 * M), bf16),
            pltpu.VMEM((M, M), bf16),
            pltpu.VMEM((2, 8, M, D), bf16),
            pltpu.VMEM((2, 8, Dc, D), bf16),
            pltpu.VMEM((2, 8, Dc, D), bf16),
            pltpu.VMEM((S, M), f32),
            pltpu.VMEM((S, 128), f32),
            pltpu.VMEM((S, D), bf16),
            pltpu.VMEM((S, D), bf16),
            pltpu.VMEM((S, D), bf16),
            pltpu.VMEM((2, BQ, S), f32),
            pltpu.VMEM((2, S // CK + 1, BQ, 128), f32),
            pltpu.VMEM((2, S // 128, BQ, 128), bf16),
            pltpu.VMEM((2, BQ, D), f32),
            pltpu.VMEM((2, BQ, D), bf16),
            pltpu.VMEM((RB + 16, M), f32),
            pltpu.VMEM((RB + 16, M), f32),
            pltpu.VMEM((NB, RB, M), bf16),
            pltpu.SemaphoreType.DMA((9 + NB,)),
        ],
        compiler_params=pltpu.CompilerParams(
            dimension_semantics=("arbitrary",),
            vmem_limit_bytes=120 * 1024 * 1024,
        ),
    )(x, c, wq, wuk, wuv, wo, B_wqkv, B_wo, gw)
    return out.reshape(B, S, M)
```

```python
import functools
import math

import jax
import jax.numpy as jnp
import numpy as np
import jax.experimental.pallas as pl
import jax.experimental.pallas.tpu as pltpu

_LOG2E = math.log2(math.e)
_NT = (((1,), (1,)), ((), ()))
_NEG = -1e9 * _LOG2E
_PACKED_LOADS = 'xcwoqkvzb'
_Q_ORDER = [3, 4, 2, 5, 1, 6, 0, 7]


def _merge(*lists):
    items = []
    for li, lst in enumerate(lists):
        n = len(lst)
        for k, t in enumerate(lst):
            items.append(((k + 0.5) / n, li, k, t))
    items.sort(key=lambda e: (e[0], e[1], e[2]))
    return [e[3] for e in items]


def _kernel(x_hbm, c_hbm, wq_hbm, wuk_hbm, wuv_hbm, wo_hbm, wqkv_hbm, wob_hbm, gw_ref,
            o_hbm,
            x_s, c_s, wq_raw, wuk_raw, wuv_raw, wo_s, wqkv_s, wt_s, wob_s,
            wq_s, wuk_s, wuv_s, acc_s, g_s, q_s, k_s, v_s, s_s, m_s, p_s, r_s, ctx_s, qb_s, kh_s, vh_s, ob_s, ostage, gw_s, sems,
            *, S, H, D, HB, DB, W, DIL, BQ, RB, CK, NC, RS, FILL_AT, CKV, NH, TS):
    step = pl.program_id(0)
    f32, bf16, u32 = jnp.float32, jnp.bfloat16, jnp.uint32
    NB = S // RB
    M = x_s.shape[0] * 128
    DM = HB * DB
    HALO = 16

    U = _PACKED_LOADS

    def ld(tag, ref, *idx):
        if tag in U:
            rows = idx[-1]
            if isinstance(rows, slice):
                rows = slice(None) if rows.start is None else slice(rows.start // 2, rows.stop // 2)
            elif isinstance(rows, pl.Slice):
                rows = pl.ds(pl.multiple_of(rows.start // 2, rows.size // 2), rows.size // 2)
            return pltpu.bitcast(ref.bitcast(u32)[idx[:-1] + (rows,)], bf16)
        return ref[idx]

    def tob(v):
        return v.astype(bf16)

    def recip(l):
        r = pl.reciprocal(l, approx=True)
        return r * (2.0 - l * r)

    def ld_tiles(tag, ref32, rows, ntile):
        return jnp.concatenate([ld(tag, ref32, t, rows) for t in range(ntile)], axis=1)

    NLT = M // 128
    HR = RB // NH

    def cp(i):
        srcs = [
            None,
            (wqkv_hbm.at[:, pl.ds(0, DM)], wqkv_s.at[0]),
            (wqkv_hbm.at[:, pl.ds(DM, DM)], wqkv_s.at[1]),
            (wqkv_hbm.at[:, pl.ds(2 * DM, DM)], wqkv_s.at[2]),
            None,
            None,
            (wuk_hbm, wuk_raw),
            (wuv_hbm, wuv_raw),
            (wq_hbm, wq_raw),
            None,
        ]
        s, d = srcs[i]
        return pltpu.make_async_copy(s, d, sems.at[i])
    NCP = 10

    def wob_cp(t):
        return pltpu.make_async_copy(wob_hbm.at[:, pl.ds(t * 128, 128)], wob_s.at[t], sems.at[NCP + t])

    def tile_cps(kind):
        base = {'x0': 0, 'x1': 1, 'c': 2, 'wo': 3}[kind] * NLT + NCP + NLT
        if kind == 'x0':
            return [pltpu.make_async_copy(x_hbm.at[pl.ds(0, HR), pl.ds(t * 128, 128)], x_s.at[t, pl.ds(0, HR)],
                                          sems.at[base + t]) for t in range(NLT)]
        if kind == 'x1':
            return [pltpu.make_async_copy(x_hbm.at[pl.ds(HR, S - HR), pl.ds(t * 128, 128)],
                                          x_s.at[t, pl.ds(HR, S - HR)], sems.at[base + t]) for t in range(NLT)]
        if kind == 'c':
            return [pltpu.make_async_copy(c_hbm.at[:, pl.ds(t * 128, 128)], c_s.at[t],
                                          sems.at[base + t]) for t in range(c_s.shape[0])]
        return [pltpu.make_async_copy(wo_hbm.at[:, pl.ds(t * 128, 128)], wo_s.at[t],
                                      sems.at[base + t]) for t in range(NLT)]
    NSEM = NCP + 5 * NLT
    M = NLT * 128

    GH = 8
    NCH = GH

    def prep_weights(grp, src_grp, ch):
        slot = grp & 1
        thunks = []
        for raw, dst in ((wq_raw, wq_s), (wuk_raw, wuk_s), (wuv_raw, wuv_s)):
            rows = dst.shape[2] // NCH
            base = pl.multiple_of(ch * (rows * (H // 2)) + src_grp * (GH // 2), GH // 2)
            d0 = pl.multiple_of(ch * rows, rows)
            for b in range(GH // 2):
                def t(raw=raw, dst=dst, rows=rows, base=base, d0=d0, b=b):
                    w32 = raw.bitcast(u32).at[pl.ds(base, rows * (H // 2) - (H - GH) // 2)][pl.ds(b, rows, stride=H // 2), :]
                    lo = pltpu.bitcast(w32 << 16, f32).astype(bf16)
                    hi = pltpu.bitcast(w32 & u32(0xFFFF0000), f32).astype(bf16)
                    dst[slot, 2 * b, pl.ds(d0, rows), :] = lo
                    dst[slot, 2 * b + 1, pl.ds(d0, rows), :] = hi
                thunks.append(t)
        return thunks

    def transpose_part(p):
        for kt in range(NLT):
            for nt in range(DM // 128):
                wt_s[kt, p * DM + nt * 128:p * DM + (nt + 1) * 128, :] = (
                    wqkv_s[p, kt * 128:(kt + 1) * 128, nt * 128:(nt + 1) * 128].T)

    def gather_rows(ref32, lead, base, c):
        parts = [ref32[lead, pl.ds(base + 2 * c + j, HB, stride=DB // 2), :] for j in range(2)]
        return pltpu.bitcast(jnp.concatenate(parts, axis=0), bf16)

    @pl.when(step == 0)
    def _():
        for d_ in tile_cps('x0'):
            d_.start()
        for i in range(1, 4):
            cp(i).start()
        gw_s[...] = gw_ref[...].astype(f32).reshape(1, M)
        for c in range(NLT):
            kh_s[c, RB:RB + HALO, :] = jnp.zeros((HALO, 128), f32)
            vh_s[c, RB:RB + HALO, :] = jnp.zeros((HALO, 128), f32)
        for d_ in tile_cps('x0'):
            d_.wait()
        cp(1).wait()
        transpose_part(0)

    @pl.when(step == 1)
    def _():
        for d_ in tile_cps('x1'):
            d_.wait()

    @pl.when(step < NB)
    def _():
        r0 = pl.multiple_of(step * RB, RB)
        wt32 = wt_s.bitcast(u32)
        wob32 = wob_s.bitcast(u32)
        for c in range(NLT):
            kh_s[c, 0:HALO, :] = kh_s[c, RB:RB + HALO, :]
            vh_s[c, 0:HALO, :] = vh_s[c, RB:RB + HALO, :]
        lane = jax.lax.broadcasted_iota(jnp.int32, (TS, 128), 1)
        odd = (lane & 1) == 1
        NG = 4

        def stage_p(hf, p):
            a0 = hf * HR
            th = []
            for c0 in range(0, NLT, NG):
                def t(c0=c0):
                    xb = ld_tiles('x', x_s, pl.ds(r0 + a0, HR), NLT)
                    w = jnp.concatenate(
                        [jnp.concatenate([gather_rows(wt32, kt, p * (DM // 2), c) for kt in range(NLT)], axis=1)
                         for c in range(c0, c0 + NG)], axis=0)
                    y = jax.lax.dot_general(xb, w, _NT, preferred_element_type=f32)
                    for c in range(c0, c0 + NG):
                        yc = y[:, (c - c0) * 128:(c - c0 + 1) * 128]
                        if p == 0:
                            qb_s[hf % 2, c] = yc * ((DB ** -0.5) * _LOG2E)
                        elif p == 1:
                            kh_s[c, HALO + a0:HALO + a0 + HR, :] = yc
                        else:
                            vh_s[c, HALO + a0:HALO + a0 + HR, :] = yc
                th.append(t)
            return th

        def stage_g(hf):
            a0 = hf * HR

            def t():
                xb = ld_tiles('x', x_s, pl.ds(r0 + a0, HR), NLT)
                z = jnp.sum(xb.astype(f32) * gw_s[...], axis=-1, keepdims=True)
                g_s[pl.ds(r0 + a0, HR), :] = jnp.broadcast_to(jax.nn.sigmoid(z), (HR, 128))
            return [t]

        def stage_t(hf):
            th = []
            for a0 in range(hf * HR, (hf + 1) * HR, TS):
                def t(a0=a0):
                    qa = a0 - hf * HR
                    tts = [None] * W
                    for c in range(NLT):
                        qc = qb_s[hf % 2, c, qa:qa + TS, :]
                        for w in range(W):
                            k0 = HALO + a0 - w * DIL
                            pr = qc * kh_s[c, k0:k0 + TS, :]
                            tts[w] = pr if c == 0 else tts[w] + pr
                    logits = []
                    for w in range(W):
                        tt = tts[w]
                        tt = tt + pltpu.roll(tt, 64, 1)
                        tt = tt + jnp.where(odd, pltpu.roll(tt, 1, 1), pltpu.roll(tt, 127, 1))
                        if w > 0 and a0 < (W - 1) * DIL:
                            pos = r0 + a0 + jax.lax.broadcasted_iota(jnp.int32, (TS, 128), 0)
                            tt = jnp.where(pos >= w * DIL, tt, _NEG)
                        logits.append(tt)
                    m = logits[0]
                    for w in range(1, W):
                        m = jnp.maximum(m, logits[w])
                    ps = [jnp.exp2(lg - m) for lg in logits]
                    l = ps[0]
                    for w in range(1, W):
                        l = l + ps[w]
                    r = (1.0 - g_s[pl.ds(r0 + a0, TS), :]) * recip(l)
                    ps = [pw * r for pw in ps]
                    for c in range(NLT):
                        o = ps[0] * vh_s[c, HALO + a0:HALO + a0 + TS, :]
                        for w in range(1, W):
                            k0 = HALO + a0 - w * DIL
                            o = o + ps[w] * vh_s[c, k0:k0 + TS, :]
                        ob_s[hf % 2, c, qa:qa + TS, :] = tob(o)
                th.append(t)
            return th

        def stage_o(hf):
            a0 = hf * HR
            th = []
            for n0 in range(0, NLT, NG):
                def t(n0=n0):
                    lhs = jnp.concatenate([ld('b', ob_s, hf % 2, c, slice(None)) for c in range(NLT)], axis=1)
                    w = jnp.concatenate(
                        [jnp.concatenate([gather_rows(wob32, nt, 0, c) for c in range(NLT)], axis=0)
                         for nt in range(n0, n0 + NG)], axis=1)
                    acc_s[pl.ds(r0 + a0, HR), n0 * 128:(n0 + NG) * 128] = jnp.dot(
                        lhs, w, preferred_element_type=f32)
                th.append(t)
            return th

        def run(ths):
            for t in ths:
                t()

        run(_merge(stage_p(0, 0), stage_g(0)))

        @pl.when(step == 0)
        def _():
            for d_ in tile_cps('x1'):
                d_.start()
            for t in range(NLT):
                wob_cp(t).start()
            for i in range(6, 9):
                cp(i).start()
            for d_ in tile_cps('c') + tile_cps('wo'):
                d_.start()
            cp(2).wait()
            transpose_part(1)
        run(stage_p(0, 1))

        @pl.when(step == 0)
        def _():
            cp(3).wait()
            transpose_part(2)
        run(stage_p(0, 2))
        for hf in range(1, NH + 2):
            lists = []
            if hf < NH:
                lists.append(stage_p(hf, 0) + stage_p(hf, 1) + stage_p(hf, 2) + stage_g(hf))
            if hf - 1 < NH:
                lists.append(stage_t(hf - 1))
            if hf >= 2:
                lists.append(stage_o(hf - 2))
            if hf == 2:
                @pl.when(step == 0)
                def _():
                    for t in range(NLT):
                        wob_cp(t).wait()
            run(_merge(*lists))

    @pl.when(step == NB - 1)
    def _():
        for i in range(6, 9):
            cp(i).wait()
        for d_ in tile_cps('c') + tile_cps('wo'):
            d_.wait()
        def body(ch, carry):
            for t in prep_weights(0, 0, ch):
                t()
            return carry
        jax.lax.fori_loop(0, NCH, body, 0)

    @pl.when(step >= NB)
    def _():
        h = step - NB
        slot = (h >> 3) & 1
        hh = h & 7
        qscale = (D ** -0.5) * _LOG2E
        xall = ld_tiles('x', x_s, slice(None), NLT)
        q_s[...] = tob(jnp.dot(xall, ld('w', wq_s, slot, hh, slice(None)), preferred_element_type=f32) * qscale)
        call = ld_tiles('c', c_s, slice(None), c_s.shape[0])
        k_s[...] = tob(jnp.dot(call, ld('w', wuk_s, slot, hh, slice(None)), preferred_element_type=f32))
        v_s[...] = tob(jnp.dot(call, ld('w', wuv_s, slot, hh, slice(None)), preferred_element_type=f32))
        wo_rows = pl.ds(pl.multiple_of(h * D, D), D)
        fill = prep_weights((h >> 3) + 1, jnp.minimum((h >> 3) + 1, H // GH - 1), hh)

        HF = BQ // 2
        row = jax.lax.broadcasted_iota(jnp.int32, (HF, HF), 0)
        col = jax.lax.broadcasted_iota(jnp.int32, (HF, HF), 1)
        cmask = col <= row
        nq = S // BQ
        st = [dict() for _ in range(nq)]

        def upd(d, key, val):
            d[key] = val if not (key in d) else d[key] + val

        def tmax(a):
            r = a[:, 0:128]
            for t in range(1, a.shape[1] // 128):
                r = jnp.maximum(r, a[:, t * 128:(t + 1) * 128])
            return r

        def ptiles(slot, a0, a1, c0, c1):
            return jnp.concatenate([ld('p', p_s, slot, c, slice(a0, a1)) for c in range(c0 // 128, c1 // 128)], axis=1)

        def stage_a(i):
            r0 = i * BQ
            th = []
            nmx = 0
            for c0 in range(0, r0, CK):
                def t(c0=c0, nmx=nmx):
                    ck = min(CK, r0 - c0)
                    s = jax.lax.dot_general(ld('q', q_s, slice(r0, r0 + BQ)), ld('k', k_s, slice(c0, c0 + ck)), _NT,
                                            preferred_element_type=f32)
                    s_s[sl[i], :, c0:c0 + ck] = s
                    m_s[sl[i], nmx] = tmax(s)
                th.append(t)
                nmx += 1

            def td1(nmx=nmx):
                s1 = jax.lax.dot_general(ld('q', q_s, slice(r0, r0 + HF)), ld('k', k_s, slice(r0, r0 + HF)), _NT,
                                         preferred_element_type=f32)
                s1 = jnp.where(cmask, s1, _NEG)
                s_s[sl[i], 0:HF, r0:r0 + HF] = s1
                m_s[sl[i], nmx, 0:HF, :] = s1

            def td2(nmx=nmx):
                s2 = jax.lax.dot_general(ld('q', q_s, slice(r0 + HF, r0 + BQ)), ld('k', k_s, slice(r0, r0 + BQ)), _NT,
                                         preferred_element_type=f32)
                s2b = jnp.where(cmask, s2[:, HF:BQ], _NEG)
                s_s[sl[i], HF:BQ, r0:r0 + HF] = s2[:, 0:HF]
                s_s[sl[i], HF:BQ, r0 + HF:r0 + BQ] = s2b
                m_s[sl[i], nmx, HF:BQ, :] = jnp.maximum(s2[:, 0:HF], s2b)
            return th + [td1, td2]

        def stage_sm(i):
            r0 = i * BQ
            th = []
            nmx = (r0 + CK - 1) // CK + 1
            for a0 in range(0, BQ, RS):
                def t(a0=a0):
                    L = r0 + (HF if a0 < HF else BQ)
                    nt = L // 128
                    m = m_s[sl[i], 0, a0:a0 + RS, :]
                    for c in range(1, nmx):
                        m = jnp.maximum(m, m_s[sl[i], c, a0:a0 + RS, :])
                    m = jnp.max(m, axis=-1, keepdims=True)
                    l = None
                    for c in range(nt):
                        p = jnp.exp2(s_s[sl[i], a0:a0 + RS, c * 128:(c + 1) * 128] - m)
                        l = p if l is None else l + p
                        p_s[sl[i], c, a0:a0 + RS, :] = tob(p)
                    l = jnp.sum(l, axis=-1, keepdims=True)
                    r_s[sl[i], a0:a0 + RS, :] = g_s[r0 + a0:r0 + a0 + RS, :] * recip(l)
                th.append(t)
            return th

        def stage_pv(i):
            r0 = i * BQ
            d = st[i]
            th = []
            for c0 in range(0, r0, CKV):
                def t(c0=c0):
                    ck = min(CKV, r0 - c0)
                    upd(d, 'o', jnp.dot(ptiles(sl[i], 0, BQ, c0, c0 + ck), ld('v', v_s, slice(c0, c0 + ck)),
                                        preferred_element_type=f32))
                th.append(t)

            def td():
                o1 = jnp.dot(ptiles(sl[i], 0, HF, r0, r0 + HF), ld('v', v_s, slice(r0, r0 + HF)), preferred_element_type=f32)
                o2 = jnp.dot(ptiles(sl[i], HF, BQ, r0, r0 + BQ), ld('v', v_s, slice(r0, r0 + BQ)), preferred_element_type=f32)
                upd(d, 'o', jnp.concatenate([o1, o2], axis=0))
                ctx_s[sl[i]] = tob(d['o'] * r_s[sl[i]])
            return th + [td]

        def stage_c(i, wo_rows=wo_rows):
            r0 = i * BQ
            th = []
            for n0 in range(0, M, NC):
                def t(n0=n0):
                    acc_s[r0:r0 + BQ, n0:n0 + NC] += jnp.dot(ld('z', ctx_s, sl[i], slice(None)), jnp.concatenate(
                        [ld('o', wo_s, t, wo_rows) for t in range(n0 // 128, (n0 + NC) // 128)], axis=1),
                                                             preferred_element_type=f32)
                th.append(t)
            return th

        prog = []
        seq = _Q_ORDER if nq == len(_Q_ORDER) else list(range(nq))
        sl = {b: n % 2 for n, b in enumerate(seq)}
        for t_ in range(nq + 3):
            lists = []
            if t_ < nq:
                lists.append(stage_a(seq[t_]))
            if 0 <= t_ - 1 < nq:
                lists.append(stage_sm(seq[t_ - 1]))
            if 0 <= t_ - 2 < nq:
                lists.append(stage_pv(seq[t_ - 2]))
            if 0 <= t_ - 3 < nq:
                lists.append(stage_c(seq[t_ - 3]))
            if t_ == FILL_AT:
                lists.append(fill)
            prog += _merge(*lists)
        for t in prog:
            t()

    @pl.when(step == NB + H - 1)
    def _():
        def ocp(b):
            return pltpu.make_async_copy(ostage.at[b], o_hbm.at[pl.ds(b * RO, RO)], sems.at[NSEM + b])
        RO = ostage.shape[1]
        for b in range(S // RO):
            ostage[b] = acc_s[b * RO:(b + 1) * RO, :].astype(bf16)
            ocp(b).start()
        for b in range(S // RO):
            ocp(b).wait()


@jax.jit
def pallas_gated_mix__compressed_kv_cla__sliding_local_dilated__prompt_kernel(
    A_x: jax.Array,
    A_c_kv: jax.Array,
    A_w_q: jax.Array,
    A_w_uk: jax.Array,
    A_w_uv: jax.Array,
    A_w_o: jax.Array,
    B_x: jax.Array,
    B_wqkv: jax.Array,
    B_wo: jax.Array,
    gate_w: jax.Array,
):
    B, S, M = A_x.shape
    _, H, D = A_w_q.shape
    Dc = A_c_kv.shape[2]
    HB = 32
    DB = M // HB
    W, DIL = 8, 2
    BQ, RO = 256, 256
    CK, CKV, NC, RS, FILL_AT, RB, NH, TS = 512, 1024, 512, 32, 5, 512, 2, 16
    NB = S // RB
    f32, bf16, u32 = jnp.float32, jnp.bfloat16, jnp.uint32

    x = A_x.reshape(S, M)
    c = A_c_kv.reshape(S, Dc)
    wq = A_w_q.reshape(M * H, D)
    wuk = A_w_uk.reshape(Dc * H, D)
    wuv = A_w_uv.reshape(Dc * H, D)
    wo = A_w_o.reshape(H * D, M)
    gw = gate_w

    hbm = pl.BlockSpec(memory_space=pltpu.HBM)
    kern = functools.partial(_kernel, S=S, H=H, D=D, HB=HB, DB=DB, W=W, DIL=DIL, BQ=BQ, RB=RB,
                             CK=CK, NC=NC, RS=RS, FILL_AT=FILL_AT, CKV=CKV, NH=NH, TS=TS)
    out = pl.pallas_call(
        kern,
        grid=(NB + H,),
        in_specs=[hbm] * 8 + [pl.BlockSpec((M,), lambda s: (0,))],
        out_specs=hbm,
        out_shape=jax.ShapeDtypeStruct((S, M), A_x.dtype),
        scratch_shapes=[
            pltpu.VMEM((M // 128, S, 128), bf16),
            pltpu.VMEM((Dc // 128, S, 128), bf16),
            pltpu.VMEM((M * H, D), bf16),
            pltpu.VMEM((Dc * H, D), bf16),
            pltpu.VMEM((Dc * H, D), bf16),
            pltpu.VMEM((M // 128, H * D, 128), bf16),
            pltpu.VMEM((3, M, M), bf16),
            pltpu.VMEM((M // 128, 3 * M, 128), bf16),
            pltpu.VMEM((M // 128, M, 128), bf16),
            pltpu.VMEM((2, 8, M, D), bf16),
            pltpu.VMEM((2, 8, Dc, D), bf16),
            pltpu.VMEM((2, 8, Dc, D), bf16),
            pltpu.VMEM((S, M), f32),
            pltpu.VMEM((S, 128), f32),
            pltpu.VMEM((S, D), bf16),
            pltpu.VMEM((S, D), bf16),
            pltpu.VMEM((S, D), bf16),
            pltpu.VMEM((2, BQ, S), f32),
            pltpu.VMEM((2, S // CK + 1, BQ, 128), f32),
            pltpu.VMEM((2, S // 128, BQ, 128), bf16),
            pltpu.VMEM((2, BQ, D), f32),
            pltpu.VMEM((2, BQ, D), bf16),
            pltpu.VMEM((2, M // 128, RB // NH, 128), f32),
            pltpu.VMEM((M // 128, RB + 16, 128), f32),
            pltpu.VMEM((M // 128, RB + 16, 128), f32),
            pltpu.VMEM((2, M // 128, RB // NH, 128), bf16),
            pltpu.VMEM((S // RO, RO, M), bf16),
            pltpu.VMEM((1, M), f32),
            pltpu.SemaphoreType.DMA((10 + 5 * (M // 128) + S // RO,)),
        ],
        compiler_params=pltpu.CompilerParams(
            dimension_semantics=("arbitrary",),
            vmem_limit_bytes=120 * 1024 * 1024,
        ),
    )(x, c, wq, wuk, wuv, wo, B_wqkv, B_wo, gw)
    return out.reshape(B, S, M)
```

```python
import functools
import math

import jax
import jax.numpy as jnp
import numpy as np
import jax.experimental.pallas as pl
import jax.experimental.pallas.tpu as pltpu

_LOG2E = math.log2(math.e)
_NT = (((1,), (1,)), ((), ()))
_NEG = -1e9 * _LOG2E
_PACKED_LOADS = 'xcwoqkvzb'
_Q_ORDER = [2, 4, 3, 5, 1, 6, 7, 0]


def _merge(*lists):
    items = []
    for li, lst in enumerate(lists):
        n = len(lst)
        for k, t in enumerate(lst):
            items.append(((k + 0.5) / n, li, k, t))
    items.sort(key=lambda e: (e[0], e[1], e[2]))
    return [e[3] for e in items]


def _kernel(x_hbm, c_hbm, wq_hbm, wuk_hbm, wuv_hbm, wo_hbm, wqkv_hbm, wob_hbm, gw_ref,
            o_hbm,
            x_s, c_s, wq_raw, wuk_raw, wuv_raw, wo_s, wqkv_s, wt_s, wob_s,
            wq_s, wuk_s, wuv_s, acc_s, g_s, q_s, k_s, v_s, s_s, m_s, p_s, r_s, ctx_s, qb_s, kh_s, vh_s, ob_s, ostage, gw_s, gwb_s, sems,
            *, S, H, D, HB, DB, W, DIL, BQ, RB, CK, NC, RS, FILL_AT, CKV, NH, TS):
    f32, bf16, u32 = jnp.float32, jnp.bfloat16, jnp.uint32
    NB = S // RB
    M = x_s.shape[0] * 128
    DM = HB * DB
    HALO = 16

    U = _PACKED_LOADS

    def ld(tag, ref, *idx):
        if tag in U:
            rows = idx[-1]
            if isinstance(rows, slice):
                rows = slice(None) if rows.start is None else slice(rows.start // 2, rows.stop // 2)
            elif isinstance(rows, pl.Slice):
                rows = pl.ds(pl.multiple_of(rows.start // 2, rows.size // 2), rows.size // 2)
            return pltpu.bitcast(ref.bitcast(u32)[idx[:-1] + (rows,)], bf16)
        return ref[idx]

    def tob(v):
        return v.astype(bf16)

    def recip(l):
        r = pl.reciprocal(l, approx=True)
        return r * (2.0 - l * r)

    def ld_tiles(tag, ref32, rows, ntile):
        return jnp.concatenate([ld(tag, ref32, t, rows) for t in range(ntile)], axis=1)

    NLT = M // 128
    HR = RB // NH

    def cp(i):
        srcs = [
            (gw_ref, gwb_s),
            (wqkv_hbm.at[:, pl.ds(0, DM)], wqkv_s.at[0]),
            (wqkv_hbm.at[:, pl.ds(DM, DM)], wqkv_s.at[1]),
            (wqkv_hbm.at[:, pl.ds(2 * DM, DM)], wqkv_s.at[2]),
            None,
            None,
            (wuk_hbm, wuk_raw),
            (wuv_hbm, wuv_raw),
            (wq_hbm, wq_raw),
            None,
        ]
        s, d = srcs[i]
        return pltpu.make_async_copy(s, d, sems.at[i])
    NCP = 10

    def wob_cp(t):
        return pltpu.make_async_copy(wob_hbm.at[:, pl.ds(t * 128, 128)], wob_s.at[t], sems.at[NCP + t])

    def tile_cps(kind):
        base = {'x0': 0, 'x1': 1, 'c': 2, 'wo': 3, 'xm': 4}[kind] * NLT + NCP + NLT
        if kind == 'x0':
            return [pltpu.make_async_copy(x_hbm.at[pl.ds(0, HR), pl.ds(t * 128, 128)], x_s.at[t, pl.ds(0, HR)],
                                          sems.at[base + t]) for t in range(NLT)]
        if kind in ('xm', 'x1'):
            a0, a1 = (HR, RB) if kind == 'xm' else (RB, S)
            return [pltpu.make_async_copy(x_hbm.at[pl.ds(a0, a1 - a0), pl.ds(t * 128, 128)],
                                          x_s.at[t, pl.ds(a0, a1 - a0)], sems.at[base + t]) for t in range(NLT)]
        if kind == 'c':
            return [pltpu.make_async_copy(c_hbm.at[:, pl.ds(t * 128, 128)], c_s.at[t],
                                          sems.at[base + t]) for t in range(c_s.shape[0])]
        return [pltpu.make_async_copy(wo_hbm.at[:, pl.ds(t * 128, 128)], wo_s.at[t],
                                      sems.at[base + t]) for t in range(NLT)]
    NSEM = NCP + 6 * NLT
    M = NLT * 128

    GH = 8
    NCH = GH

    def prep_weights(grp, src_grp, ch):
        slot = grp & 1
        thunks = []
        for raw, dst in ((wq_raw, wq_s), (wuk_raw, wuk_s), (wuv_raw, wuv_s)):
            rows = dst.shape[2] // NCH
            base = pl.multiple_of(ch * (rows * (H // 2)) + src_grp * (GH // 2), GH // 2)
            d0 = pl.multiple_of(ch * rows, rows)
            for b in range(GH // 2):
                def t(raw=raw, dst=dst, rows=rows, base=base, d0=d0, b=b):
                    w32 = raw.bitcast(u32).at[pl.ds(base, rows * (H // 2) - (H - GH) // 2)][pl.ds(b, rows, stride=H // 2), :]
                    lo = pltpu.bitcast(w32 << 16, f32).astype(bf16)
                    hi = pltpu.bitcast(w32 & u32(0xFFFF0000), f32).astype(bf16)
                    dst[slot, 2 * b, pl.ds(d0, rows), :] = lo
                    dst[slot, 2 * b + 1, pl.ds(d0, rows), :] = hi
                thunks.append(t)
        return thunks

    def transpose_part(p):
        for kt in range(NLT):
            for nt in range(DM // 128):
                wt_s[kt, p * DM + nt * 128:p * DM + (nt + 1) * 128, :] = (
                    wqkv_s[p, kt * 128:(kt + 1) * 128, nt * 128:(nt + 1) * 128].T)

    def gather_rows(ref32, lead, base, c):
        parts = [ref32[lead, pl.ds(base + 2 * c + j, HB, stride=DB // 2), :] for j in range(2)]
        return pltpu.bitcast(jnp.concatenate(parts, axis=0), bf16)

    if True:
        for d_ in tile_cps('x0'):
            d_.start()
        for i in range(0, 2):
            cp(i).start()
        for c in range(NLT):
            kh_s[c, RB:RB + HALO, :] = jnp.zeros((HALO, 128), f32)
            vh_s[c, RB:RB + HALO, :] = jnp.zeros((HALO, 128), f32)
        cp(0).wait()
        gw_s[...] = gwb_s[...].astype(f32).reshape(1, M)
        for d_ in tile_cps('x0'):
            d_.wait()
        cp(1).wait()
        cp(2).start()
        cp(3).start()
        for d_ in tile_cps('xm'):
            d_.start()
        transpose_part(0)

    def b_step(step, carry):
        @pl.when(step == 1)
        def _():
            for d_ in tile_cps('x1'):
                d_.wait()

        r0 = pl.multiple_of(step * RB, RB)
        wt32 = wt_s.bitcast(u32)
        wob32 = wob_s.bitcast(u32)
        for c in range(NLT):
            kh_s[c, 0:HALO, :] = kh_s[c, RB:RB + HALO, :]
            vh_s[c, 0:HALO, :] = vh_s[c, RB:RB + HALO, :]
        lane = jax.lax.broadcasted_iota(jnp.int32, (TS, 128), 1)
        odd = (lane & 1) == 1
        NG = 2

        def stage_p(hf, p):
            a0 = hf * HR
            th = []
            for c0 in range(0, NLT, NG):
                def t(c0=c0):
                    xb = ld_tiles('x', x_s, pl.ds(r0 + a0, HR), NLT)
                    w = jnp.concatenate(
                        [jnp.concatenate([gather_rows(wt32, kt, p * (DM // 2), c) for kt in range(NLT)], axis=1)
                         for c in range(c0, c0 + NG)], axis=0)
                    y = jax.lax.dot_general(xb, w, _NT, preferred_element_type=f32)
                    for c in range(c0, c0 + NG):
                        yc = y[:, (c - c0) * 128:(c - c0 + 1) * 128]
                        if p == 0:
                            qb_s[hf % 2, c] = yc * ((DB ** -0.5) * _LOG2E)
                        elif p == 1:
                            kh_s[c, HALO + a0:HALO + a0 + HR, :] = yc
                        else:
                            vh_s[c, HALO + a0:HALO + a0 + HR, :] = yc
                th.append(t)
            return th

        def stage_g(hf):
            a0 = hf * HR

            def t():
                xb = ld_tiles('x', x_s, pl.ds(r0 + a0, HR), NLT)
                z = jnp.sum(xb.astype(f32) * gw_s[...], axis=-1, keepdims=True)
                g_s[pl.ds(r0 + a0, HR), :] = jnp.broadcast_to(jax.nn.sigmoid(z), (HR, 128))
            return [t]

        def stage_t(hf):
            th = []
            for a0 in range(hf * HR, (hf + 1) * HR, TS):
                def t(a0=a0):
                    qa = a0 - hf * HR
                    tts = [None] * W
                    for c in range(NLT):
                        qc = qb_s[hf % 2, c, qa:qa + TS, :]
                        for w in range(W):
                            k0 = HALO + a0 - w * DIL
                            pr = qc * kh_s[c, k0:k0 + TS, :]
                            tts[w] = pr if c == 0 else tts[w] + pr
                    logits = []
                    for w in range(W):
                        tt = tts[w]
                        tt = tt + pltpu.roll(tt, 64, 1)
                        tt = tt + jnp.where(odd, pltpu.roll(tt, 1, 1), pltpu.roll(tt, 127, 1))
                        if w > 0 and a0 < (W - 1) * DIL:
                            pos = r0 + a0 + jax.lax.broadcasted_iota(jnp.int32, (TS, 128), 0)
                            tt = jnp.where(pos >= w * DIL, tt, _NEG)
                        logits.append(tt)
                    m = logits[0]
                    for w in range(1, W):
                        m = jnp.maximum(m, logits[w])
                    ps = [jnp.exp2(lg - m) for lg in logits]
                    l = ps[0]
                    for w in range(1, W):
                        l = l + ps[w]
                    r = (1.0 - g_s[pl.ds(r0 + a0, TS), :]) * recip(l)
                    ps = [pw * r for pw in ps]
                    for c in range(NLT):
                        o = ps[0] * vh_s[c, HALO + a0:HALO + a0 + TS, :]
                        for w in range(1, W):
                            k0 = HALO + a0 - w * DIL
                            o = o + ps[w] * vh_s[c, k0:k0 + TS, :]
                        ob_s[hf % 2, c, qa:qa + TS, :] = tob(o)
                th.append(t)
            return th

        def stage_o(hf):
            a0 = hf * HR
            th = []
            for n0 in range(0, NLT, NG):
                def t(n0=n0):
                    lhs = jnp.concatenate([ld('b', ob_s, hf % 2, c, slice(None)) for c in range(NLT)], axis=1)
                    w = jnp.concatenate(
                        [jnp.concatenate([gather_rows(wob32, nt, 0, c) for c in range(NLT)], axis=0)
                         for nt in range(n0, n0 + NG)], axis=1)
                    acc_s[pl.ds(r0 + a0, HR), n0 * 128:(n0 + NG) * 128] = jnp.dot(
                        lhs, w, preferred_element_type=f32)
                th.append(t)
            return th

        def run(ths):
            for t in ths:
                t()

        run(_merge(stage_p(0, 0), stage_g(0)))

        @pl.when(step == 0)
        def _():
            cp(2).wait()
            transpose_part(1)
        run(stage_p(0, 1))

        @pl.when(step == 0)
        def _():
            cp(3).wait()
            for d_ in tile_cps('xm'):
                d_.wait()
            for t in range(NLT):
                wob_cp(t).start()
            for d_ in tile_cps('x1'):
                d_.start()
            for i in range(6, 9):
                cp(i).start()
            for d_ in tile_cps('c') + tile_cps('wo'):
                d_.start()
            transpose_part(2)
        run(stage_p(0, 2))
        for hf in range(1, NH + 2):
            lists = []
            if hf < NH:
                lists.append(stage_p(hf, 0) + stage_p(hf, 1) + stage_p(hf, 2) + stage_g(hf))
            if hf - 1 < NH:
                lists.append(stage_t(hf - 1))
            if hf >= 2:
                lists.append(stage_o(hf - 2))
            if hf == 2:
                @pl.when(step == 0)
                def _():
                    for t in range(NLT):
                        wob_cp(t).wait()
            run(_merge(*lists))

        return carry

    jax.lax.fori_loop(0, NB, b_step, 0)

    if True:
        for i in range(6, 9):
            cp(i).wait()
        for d_ in tile_cps('c') + tile_cps('wo'):
            d_.wait()
        def body(ch, carry):
            for t in prep_weights(0, 0, ch):
                t()
            return carry
        jax.lax.fori_loop(0, NCH, body, 0)

    def a_step(h, carry):
        slot = (h >> 3) & 1
        hh = h & 7
        qscale = (D ** -0.5) * _LOG2E
        xall = ld_tiles('x', x_s, slice(None), NLT)
        q_s[...] = tob(jnp.dot(xall, ld('w', wq_s, slot, hh, slice(None)), preferred_element_type=f32) * qscale)
        call = ld_tiles('c', c_s, slice(None), c_s.shape[0])
        k_s[...] = tob(jnp.dot(call, ld('w', wuk_s, slot, hh, slice(None)), preferred_element_type=f32))
        v_s[...] = tob(jnp.dot(call, ld('w', wuv_s, slot, hh, slice(None)), preferred_element_type=f32))
        wo_rows = pl.ds(pl.multiple_of(h * D, D), D)
        fill = prep_weights((h >> 3) + 1, jnp.minimum((h >> 3) + 1, H // GH - 1), hh)

        HF = BQ // 2
        row = jax.lax.broadcasted_iota(jnp.int32, (HF, HF), 0)
        col = jax.lax.broadcasted_iota(jnp.int32, (HF, HF), 1)
        cmask = col <= row
        nq = S // BQ
        st = [dict() for _ in range(nq)]

        def upd(d, key, val):
            d[key] = val if not (key in d) else d[key] + val

        def tmax(a):
            r = a[:, 0:128]
            for t in range(1, a.shape[1] // 128):
                r = jnp.maximum(r, a[:, t * 128:(t + 1) * 128])
            return r

        def ptiles(slot, a0, a1, c0, c1):
            return jnp.concatenate([ld('p', p_s, slot, c, slice(a0, a1)) for c in range(c0 // 128, c1 // 128)], axis=1)

        def stage_a(i):
            r0 = i * BQ
            th = []
            nmx = 0
            for c0 in range(0, r0, CK):
                def t(c0=c0, nmx=nmx):
                    ck = min(CK, r0 - c0)
                    s = jax.lax.dot_general(ld('q', q_s, slice(r0, r0 + BQ)), ld('k', k_s, slice(c0, c0 + ck)), _NT,
                                            preferred_element_type=f32)
                    s_s[sl[i], :, c0:c0 + ck] = s
                    m_s[sl[i], nmx] = tmax(s)
                th.append(t)
                nmx += 1

            def td1(nmx=nmx):
                s1 = jax.lax.dot_general(ld('q', q_s, slice(r0, r0 + HF)), ld('k', k_s, slice(r0, r0 + HF)), _NT,
                                         preferred_element_type=f32)
                s1 = jnp.where(cmask, s1, _NEG)
                s_s[sl[i], 0:HF, r0:r0 + HF] = s1
                m_s[sl[i], nmx, 0:HF, :] = s1

            def td2(nmx=nmx):
                s2 = jax.lax.dot_general(ld('q', q_s, slice(r0 + HF, r0 + BQ)), ld('k', k_s, slice(r0, r0 + BQ)), _NT,
                                         preferred_element_type=f32)
                s2b = jnp.where(cmask, s2[:, HF:BQ], _NEG)
                s_s[sl[i], HF:BQ, r0:r0 + HF] = s2[:, 0:HF]
                s_s[sl[i], HF:BQ, r0 + HF:r0 + BQ] = s2b
                m_s[sl[i], nmx, HF:BQ, :] = jnp.maximum(s2[:, 0:HF], s2b)
            return th + [td1, td2]

        def stage_sm(i):
            r0 = i * BQ
            th = []
            nmx = (r0 + CK - 1) // CK + 1
            for a0 in range(0, BQ, RS):
                def t(a0=a0):
                    L = r0 + (HF if a0 < HF else BQ)
                    nt = L // 128
                    m = m_s[sl[i], 0, a0:a0 + RS, :]
                    for c in range(1, nmx):
                        m = jnp.maximum(m, m_s[sl[i], c, a0:a0 + RS, :])
                    m = jnp.max(m, axis=-1, keepdims=True)
                    l = None
                    for c in range(nt):
                        p = jnp.exp2(s_s[sl[i], a0:a0 + RS, c * 128:(c + 1) * 128] - m)
                        l = p if l is None else l + p
                        p_s[sl[i], c, a0:a0 + RS, :] = tob(p)
                    l = jnp.sum(l, axis=-1, keepdims=True)
                    r_s[sl[i], a0:a0 + RS, :] = g_s[r0 + a0:r0 + a0 + RS, :] * recip(l)
                th.append(t)
            return th

        def stage_pv(i):
            r0 = i * BQ
            d = st[i]
            th = []
            for c0 in range(0, r0, CKV):
                def t(c0=c0):
                    ck = min(CKV, r0 - c0)
                    upd(d, 'o', jnp.dot(ptiles(sl[i], 0, BQ, c0, c0 + ck), ld('v', v_s, slice(c0, c0 + ck)),
                                        preferred_element_type=f32))
                th.append(t)

            def td():
                o1 = jnp.dot(ptiles(sl[i], 0, HF, r0, r0 + HF), ld('v', v_s, slice(r0, r0 + HF)), preferred_element_type=f32)
                o2 = jnp.dot(ptiles(sl[i], HF, BQ, r0, r0 + BQ), ld('v', v_s, slice(r0, r0 + BQ)), preferred_element_type=f32)
                upd(d, 'o', jnp.concatenate([o1, o2], axis=0))
                ctx_s[sl[i]] = tob(d['o'] * r_s[sl[i]])
            return th + [td]

        def stage_c(i, wo_rows=wo_rows):
            r0 = i * BQ
            th = []
            for n0 in range(0, M, NC):
                def t(n0=n0):
                    acc_s[r0:r0 + BQ, n0:n0 + NC] += jnp.dot(ld('z', ctx_s, sl[i], slice(None)), jnp.concatenate(
                        [ld('o', wo_s, t, wo_rows) for t in range(n0 // 128, (n0 + NC) // 128)], axis=1),
                                                             preferred_element_type=f32)
                th.append(t)
            return th

        prog = []
        seq = _Q_ORDER if nq == len(_Q_ORDER) else list(range(nq))
        sl = {b: n % 2 for n, b in enumerate(seq)}
        for t_ in range(nq + 3):
            lists = []
            if t_ < nq:
                lists.append(stage_a(seq[t_]))
            if 0 <= t_ - 1 < nq:
                lists.append(stage_sm(seq[t_ - 1]))
            if 0 <= t_ - 2 < nq:
                lists.append(stage_pv(seq[t_ - 2]))
            if 0 <= t_ - 3 < nq:
                lists.append(stage_c(seq[t_ - 3]))
            if t_ == FILL_AT:
                lists.append(fill)
            prog += _merge(*lists)
        for t in prog:
            t()

        return carry

    jax.lax.fori_loop(0, H, a_step, 0)

    if True:
        def ocp(b):
            return pltpu.make_async_copy(ostage.at[b], o_hbm.at[pl.ds(b * RO, RO)], sems.at[NSEM + b])
        RO = ostage.shape[1]
        for b in range(S // RO):
            ostage[b] = acc_s[b * RO:(b + 1) * RO, :].astype(bf16)
            ocp(b).start()
        for b in range(S // RO):
            ocp(b).wait()


@jax.jit
def pallas_gated_mix__compressed_kv_cla__sliding_local_dilated__prompt_kernel(
    A_x: jax.Array,
    A_c_kv: jax.Array,
    A_w_q: jax.Array,
    A_w_uk: jax.Array,
    A_w_uv: jax.Array,
    A_w_o: jax.Array,
    B_x: jax.Array,
    B_wqkv: jax.Array,
    B_wo: jax.Array,
    gate_w: jax.Array,
):
    B, S, M = A_x.shape
    _, H, D = A_w_q.shape
    Dc = A_c_kv.shape[2]
    HB = 32
    DB = M // HB
    W, DIL = 8, 2
    BQ, RO = 256, 256
    CK, CKV, NC, RS, FILL_AT, RB, NH, TS = 512, 512, 512, 32, 5, 512, 2, 16
    NB = S // RB
    f32, bf16, u32 = jnp.float32, jnp.bfloat16, jnp.uint32

    x = A_x.reshape(S, M)
    c = A_c_kv.reshape(S, Dc)
    wq = A_w_q.reshape(M * H, D)
    wuk = A_w_uk.reshape(Dc * H, D)
    wuv = A_w_uv.reshape(Dc * H, D)
    wo = A_w_o.reshape(H * D, M)
    gw = gate_w

    hbm = pl.BlockSpec(memory_space=pltpu.HBM)
    kern = functools.partial(_kernel, S=S, H=H, D=D, HB=HB, DB=DB, W=W, DIL=DIL, BQ=BQ, RB=RB,
                             CK=CK, NC=NC, RS=RS, FILL_AT=FILL_AT, CKV=CKV, NH=NH, TS=TS)
    out = pl.pallas_call(
        kern,
        in_specs=[hbm] * 9,
        out_specs=hbm,
        out_shape=jax.ShapeDtypeStruct((S, M), A_x.dtype),
        scratch_shapes=[
            pltpu.VMEM((M // 128, S, 128), bf16),
            pltpu.VMEM((Dc // 128, S, 128), bf16),
            pltpu.VMEM((M * H, D), bf16),
            pltpu.VMEM((Dc * H, D), bf16),
            pltpu.VMEM((Dc * H, D), bf16),
            pltpu.VMEM((M // 128, H * D, 128), bf16),
            pltpu.VMEM((3, M, M), bf16),
            pltpu.VMEM((M // 128, 3 * M, 128), bf16),
            pltpu.VMEM((M // 128, M, 128), bf16),
            pltpu.VMEM((2, 8, M, D), bf16),
            pltpu.VMEM((2, 8, Dc, D), bf16),
            pltpu.VMEM((2, 8, Dc, D), bf16),
            pltpu.VMEM((S, M), f32),
            pltpu.VMEM((S, 128), f32),
            pltpu.VMEM((S, D), bf16),
            pltpu.VMEM((S, D), bf16),
            pltpu.VMEM((S, D), bf16),
            pltpu.VMEM((2, BQ, S), f32),
            pltpu.VMEM((2, S // CK + 1, BQ, 128), f32),
            pltpu.VMEM((2, S // 128, BQ, 128), bf16),
            pltpu.VMEM((2, BQ, D), f32),
            pltpu.VMEM((2, BQ, D), bf16),
            pltpu.VMEM((2, M // 128, RB // NH, 128), f32),
            pltpu.VMEM((M // 128, RB + 16, 128), f32),
            pltpu.VMEM((M // 128, RB + 16, 128), f32),
            pltpu.VMEM((2, M // 128, RB // NH, 128), bf16),
            pltpu.VMEM((S // RO, RO, M), bf16),
            pltpu.VMEM((1, M), f32),
            pltpu.VMEM((M,), bf16),
            pltpu.SemaphoreType.DMA((10 + 6 * (M // 128) + S // RO,)),
        ],
        compiler_params=pltpu.CompilerParams(
            vmem_limit_bytes=120 * 1024 * 1024,
        ),
    )(x, c, wq, wuk, wuv, wo, B_wqkv, B_wo, gw)
    return out.reshape(B, S, M)
```
